```python
import os as _os
_os.environ.setdefault("JAX_PLATFORMS", "cpu")
import jax
import jax.numpy as jnp

def _softmax(x, axis=-1):
    return jax.nn.softmax(x, axis=axis)
def _gelu(x):
    return jax.nn.gelu(x, approximate=True)
def _silu(x):
    return jax.nn.silu(x)
def _sigmoid(x):
    return jax.nn.sigmoid(x)
def _layernorm(x, axis=-1, eps=1e-5):
    m = jnp.mean(x, axis=axis, keepdims=True)
    v = jnp.var(x, axis=axis, keepdims=True)
    return (x - m) / jnp.sqrt(v + eps)
def _scatter_add(tgt, idx, src, axis=0):
    return tgt.at[idx].add(src)
def _segment_sum(src, seg, n):
    return jax.ops.segment_sum(src, seg, n)
class _Rng:
    def __init__(self, key):
        self._k = key
    def _next(self):
        self._k, sub = jax.random.split(self._k)
        return sub
    def normal(self, shape):
        return jax.random.normal(self._next(), shape, dtype=jnp.bfloat16)
    def randint(self, lo, hi, shape):
        return jax.random.randint(self._next(), shape, lo, hi, dtype=jnp.int32)
    def uniform(self, shape, lo=0.0, hi=1.0):
        return jax.random.uniform(self._next(), shape, jnp.bfloat16, lo, hi)
    def permutation(self, n):
        return jax.random.permutation(self._next(), n)


kernel_name = 'standalone__gqa_block_cached__near_ridge'

def setup_inputs():
    _rng = _Rng(jax.random.key(int.from_bytes(__import__("os").urandom(4), "little")))
    _w = (lambda a: (lambda t: t.astype(jnp.bfloat16) if jnp.issubdtype(t.dtype, jnp.floating) else t)(jnp.asarray(a)))
    B, Sq, D = 8, 80, 512
    Hq, Hkv, Sk, Dh = 32, 8, 2048, 128
    assert Hq % Hkv == 0, (Hq, Hkv)
    return {
        "x": _w((lambda *s: _rng.normal(s) * 0.8)(B, Sq, D)),
        "k_cache": _w((lambda *s: _rng.normal(s) * 0.8)(B, Hkv, Sk, Dh)),
        "v_cache": _w((lambda *s: _rng.normal(s) * 0.05)(B, Hkv, Sk, Dh)),
        "wq": _w((lambda *s: _rng.normal(s) * 0.8)(D, Hq * Dh) * (D ** -0.5)),
        "wo": _w((lambda *s: _rng.normal(s) * 0.05)(Hq * Dh, D) * ((Hq * Dh) ** -0.5)),
    }

def reference(x, k_cache, v_cache, wq, wo):
    B, Sq, D = x.shape
    Hq, Dh = 32, 128
    Hkv = k_cache.shape[1]
    rep = Hq // Hkv
    q = (lambda x, *d: x.transpose(*d))((x @ wq).reshape(B, Sq, Hq, Dh), 0, 2, 1, 3)
    k = jnp.repeat(k_cache, rep, axis=1)
    v = jnp.repeat(v_cache, rep, axis=1)
    scores = jnp.einsum("bhqd,bhkd->bhqk", q, k) * (Dh ** -0.5)
    p = _softmax(scores, axis=-1)
    o = jnp.einsum("bhqk,bhkd->bhqd", p, v)
    return (lambda x, *d: x.transpose(*d))(o, 0, 2, 1, 3).reshape(B, Sq, Hq * Dh) @ wo
```

```python
import functools
import math

import jax
import jax.numpy as jnp
import jax.experimental.pallas as pl
import jax.experimental.pallas.tpu as pltpu


def _kernel(x_ref, k_ref, v_ref, wq_ref, wo_ref, out_ref, q_scr, o_scr, acc_scr,
            *, B, Sq, rep, Dh, Hkv):
    h = pl.program_id(0)
    b = pl.program_id(1)
    qscale = (Dh ** -0.5) * math.log2(math.e)

    @pl.when(b == 0)
    def _():
        q = jnp.dot(x_ref[...], wq_ref[...], preferred_element_type=jnp.float32)
        q = q * qscale
        for bb in range(B):
            for r in range(rep):
                q_scr[bb, r * Sq:(r + 1) * Sq, :] = (
                    q[bb * Sq:(bb + 1) * Sq, r * Dh:(r + 1) * Dh].astype(jnp.bfloat16))

    q = q_scr[b]
    k = k_ref[0, 0]
    v = v_ref[0, 0]
    s = jax.lax.dot_general(q, k, (((1,), (1,)), ((), ())),
                            preferred_element_type=jnp.float32)
    m = jnp.max(s, axis=-1, keepdims=True)
    p = jnp.exp2(s - m)
    l = jnp.sum(p, axis=-1, keepdims=True)
    o = jnp.dot(p.astype(jnp.bfloat16), v, preferred_element_type=jnp.float32)
    o = o / l
    row0 = pl.multiple_of(b * Sq, 16)
    for r in range(rep):
        o_scr[pl.ds(row0, Sq), r * Dh:(r + 1) * Dh] = (
            o[r * Sq:(r + 1) * Sq, :].astype(jnp.bfloat16))

    @pl.when(b == B - 1)
    def _():
        contrib = jnp.dot(o_scr[...], wo_ref[...], preferred_element_type=jnp.float32)

        @pl.when(h == 0)
        def _():
            acc_scr[...] = contrib

        @pl.when(h > 0)
        def _():
            acc_scr[...] += contrib

        @pl.when(h == Hkv - 1)
        def _():
            out_ref[...] = acc_scr[...].astype(out_ref.dtype)


@jax.jit
def pallas_standalone__gqa_block_cached__near_ridge_kernel(
    x: jax.Array,
    k_cache: jax.Array,
    v_cache: jax.Array,
    wq: jax.Array,
    wo: jax.Array,
):
    B, Sq, D = x.shape
    _, Hkv, Sk, Dh = k_cache.shape
    Hq = wq.shape[1] // Dh
    rep = Hq // Hkv
    G = rep * Dh
    x2 = x.reshape(B * Sq, D)

    kernel = functools.partial(_kernel, B=B, Sq=Sq, rep=rep, Dh=Dh, Hkv=Hkv)
    out = pl.pallas_call(
        kernel,
        grid=(Hkv, B),
        in_specs=[
            pl.BlockSpec((B * Sq, D), lambda h, b: (0, 0)),
            pl.BlockSpec((1, 1, Sk, Dh), lambda h, b: (b, h, 0, 0)),
            pl.BlockSpec((1, 1, Sk, Dh), lambda h, b: (b, h, 0, 0)),
            pl.BlockSpec((D, G), lambda h, b: (0, h)),
            pl.BlockSpec((G, D), lambda h, b: (h, 0)),
        ],
        out_specs=pl.BlockSpec((B * Sq, D), lambda h, b: (0, 0)),
        out_shape=jax.ShapeDtypeStruct((B * Sq, D), x.dtype),
        scratch_shapes=[
            pltpu.VMEM((B, rep * Sq, Dh), jnp.bfloat16),
            pltpu.VMEM((B * Sq, G), jnp.bfloat16),
            pltpu.VMEM((B * Sq, D), jnp.float32),
        ],
        compiler_params=pltpu.CompilerParams(
            dimension_semantics=("arbitrary", "arbitrary"),
            vmem_limit_bytes=64 * 1024 * 1024,
        ),
    )(x2, k_cache, v_cache, wq, wo)
    return out.reshape(B, Sq, D)
```

```python
import functools
import math

import jax
import jax.numpy as jnp
from jax import lax
import jax.experimental.pallas as pl
import jax.experimental.pallas.tpu as pltpu


def _kernel(x_hbm, k_hbm, v_hbm, wq_hbm, wo_hbm, out_ref,
            x_v, wq_v, wo_v, q_all, kbuf, vbuf, acc_scr, p0, p1,
            xsem, wqsem, wosem, ksem, vsem,
            *, B, Sq, rep, Dh, Hkv, Sk, rb, cuts, order):
    h = pl.program_id(0)
    n = B
    M = rep * Sq
    G = rep * Dh
    NC = Sk // Dh
    qscale = (Dh ** -0.5) * math.log2(math.e)
    p_bufs = (p0, p1)
    never = h < 0
    slot = lax.rem(h, 2)

    def wq_copy(hh):
        return pltpu.make_async_copy(
            wq_hbm.at[:, pl.ds(hh * G, G)], wq_v.at[hh], wqsem.at[hh])

    def wo_copy(hh, sl):
        return pltpu.make_async_copy(
            wo_hbm.at[pl.ds(hh * G, G), :], wo_v.at[sl], wosem.at[sl])

    def k_copy(hh, sl):
        return pltpu.make_async_copy(k_hbm.at[:, hh], kbuf.at[sl], ksem.at[sl])

    def v_copy(hh, sl):
        return pltpu.make_async_copy(v_hbm.at[:, hh], vbuf.at[sl], vsem.at[sl])

    @pl.when(h == 0)
    def _():
        xc = pltpu.make_async_copy(x_hbm, x_v, xsem.at[0])
        xc.start()
        wq_copy(0).start()
        wq_copy(1).start()
        xc.wait()
        for hh in range(Hkv):
            wq_copy(hh).wait()
            if hh + 2 < Hkv:
                wq_copy(hh + 2).start()
            pltpu.make_async_copy(k_hbm.at[hh, 0], kbuf.at[0, hh], ksem.at[0]).start()
            pltpu.make_async_copy(v_hbm.at[hh, 0], vbuf.at[0, hh], vsem.at[0]).start()
            if hh == Hkv - 2:
                wo_copy(0, 0).start()
            q = jnp.dot(x_v[...], wq_v[hh], preferred_element_type=jnp.float32)
            q = q * qscale
            for bb in range(B):
                for r in range(rep):
                    q_all[hh, bb, r * Sq:(r + 1) * Sq, :] = (
                        q[bb * Sq:(bb + 1) * Sq, r * Dh:(r + 1) * Dh].astype(jnp.bfloat16))

    k_copy(h, slot).wait()
    v_copy(h, slot).wait()
    wo_copy(h, slot).wait()

    @pl.when(h + 1 < Hkv)
    def _():
        k_copy(h + 1, 1 - slot).start()
        v_copy(h + 1, 1 - slot).start()
        wo_copy(h + 1, 1 - slot).start()

    def qk(i):
        q = q_all[h, i]
        k = kbuf[slot, i]
        return jax.lax.dot_general(q, k, (((1,), (1,)), ((), ())),
                                   preferred_element_type=jnp.float32)

    def sm_pv(i, s_all, dep):
        p_ref = p_bufs[i % 2]
        cut = cuts[i]
        ls = []
        part_prev = None
        full_prev = None
        full_prev2 = None
        for j in range(M // rb):
            s = s_all[j * rb:(j + 1) * rb, :]
            m = jnp.max(s, axis=-1, keepdims=True)
            m = jnp.broadcast_to(m, (rb, Dh))
            if part_prev is not None:
                m = jnp.where(never, part_prev, m)
            if full_prev2 is not None and cut < NC:
                m = jnp.where(never, full_prev2 + part_prev, m)
            ps = [jnp.exp2(s[:, c * Dh:(c + 1) * Dh] - m) for c in range(NC)]
            lp = ps[0]
            for c in range(1, NC):
                lp = lp + ps[c]
                if c == cut - 1:
                    part_prev = lp
            full_prev2 = full_prev
            full_prev = lp
            if dep is not None:
                lp = jnp.where(never, dep[j * rb:(j + 1) * rb, :], lp)
            l = jnp.sum(lp, axis=-1, keepdims=True)
            l = jnp.broadcast_to(l, (rb, Dh))
            r = pl.reciprocal(l, approx=True)
            r = r * (2.0 - l * r)
            ls.append(r)
            pb = jnp.concatenate(ps, axis=1).astype(jnp.bfloat16)
            p_ref[j * rb:(j + 1) * rb, :] = pb
        linv = jnp.concatenate(ls, axis=0)
        v = vbuf[slot, i]
        o_raw = jnp.dot(p_ref[...], v, preferred_element_type=jnp.float32)
        o = (o_raw * linv).astype(jnp.bfloat16)
        o = jnp.concatenate([o[r * Sq:(r + 1) * Sq, :] for r in range(rep)], axis=1)
        return o_raw, o

    def op(i, o):
        contrib = jnp.dot(o, wo_v[slot], preferred_element_type=jnp.float32)
        prev = acc_scr[i * Sq:(i + 1) * Sq, :]
        new = contrib + jnp.where(h > 0, prev, 0.0)
        acc_scr[i * Sq:(i + 1) * Sq, :] = new
        out_ref[i * Sq:(i + 1) * Sq, :] = new.astype(out_ref.dtype)

    s = {}
    o = {}
    oraw = {}
    s[0] = qk(0)
    if order == 0:
        for i in range(n):
            if i + 1 < n:
                s[i + 1] = qk(i + 1)
                dep = s[i + 1][:, Sk - Dh:]
            else:
                dep = oraw.get(i - 1)
            if i >= 1 and i + 1 < n:
                op(i - 1, o[i - 1])
            oraw[i], o[i] = sm_pv(i, s[i], dep)
        op(n - 2, o[n - 2])
        op(n - 1, o[n - 1])
    else:
        for i in range(n):
            if i + 1 < n:
                s[i + 1] = qk(i + 1)
                dep = s[i + 1][:, Sk - Dh:]
            else:
                dep = oraw.get(i - 1)
            oraw[i], o[i] = sm_pv(i, s[i], dep)
            if i >= 1:
                op(i - 1, o[i - 1])
        op(n - 1, o[n - 1])


def make_kernel(rb=8, cuts=None, order=1):
  @jax.jit
  def pallas_standalone__gqa_block_cached__near_ridge_kernel(
    x: jax.Array,
    k_cache: jax.Array,
    v_cache: jax.Array,
    wq: jax.Array,
    wo: jax.Array,
  ):
    B, Sq, D = x.shape
    _, Hkv, Sk, Dh = k_cache.shape
    Hq = wq.shape[1] // Dh
    rep = Hq // Hkv
    G = rep * Dh
    M = rep * Sq
    x2 = x.reshape(B * Sq, D)
    cts = cuts if cuts is not None else [10] + [16] * (B - 1)

    kernel = functools.partial(_kernel, B=B, Sq=Sq, rep=rep, Dh=Dh, Hkv=Hkv, Sk=Sk, rb=rb, cuts=cts, order=order)
    pshape = pltpu.VMEM((M, Sk), jnp.bfloat16)
    anyspec = pl.BlockSpec(memory_space=pl.ANY)
    out = pl.pallas_call(
        kernel,
        grid=(Hkv,),
        in_specs=[anyspec] * 5,
        out_specs=pl.BlockSpec((B * Sq, D), lambda h: (0, 0)),
        out_shape=jax.ShapeDtypeStruct((B * Sq, D), x.dtype),
        scratch_shapes=[
            pltpu.VMEM((B * Sq, D), jnp.bfloat16),
            pltpu.VMEM((Hkv, D, G), jnp.bfloat16),
            pltpu.VMEM((2, G, D), jnp.bfloat16),
            pltpu.VMEM((Hkv, B, M, Dh), jnp.bfloat16),
            pltpu.VMEM((2, B, Sk, Dh), jnp.bfloat16),
            pltpu.VMEM((2, B, Sk, Dh), jnp.bfloat16),
            pltpu.VMEM((B * Sq, D), jnp.float32),
            pshape, pshape,
            pltpu.SemaphoreType.DMA((1,)),
            pltpu.SemaphoreType.DMA((Hkv,)),
            pltpu.SemaphoreType.DMA((2,)),
            pltpu.SemaphoreType.DMA((2,)),
            pltpu.SemaphoreType.DMA((2,)),
        ],
        compiler_params=pltpu.CompilerParams(
            dimension_semantics=("arbitrary",),
            vmem_limit_bytes=100 * 1024 * 1024,
        ),
    )(x2, k_cache, v_cache, wq, wo)
    return out.reshape(B, Sq, D)
  return pallas_standalone__gqa_block_cached__near_ridge_kernel


pallas_standalone__gqa_block_cached__near_ridge_kernel = make_kernel()
```

```python
import functools
import math

import jax
import jax.numpy as jnp
from jax import lax
import jax.experimental.pallas as pl
import jax.experimental.pallas.tpu as pltpu


def _kernel(x_hbm, k_hbm, v_hbm, wq_hbm, wo_hbm, out_hbm,
            x_v, wq_v, wo_v, q_all, kbuf, vbuf, acc_scr, obuf, p0, p1,
            xsem, wqsem, wosem, ksem, vsem, k0sem, v0sem, osem,
            *, B, Sq, rep, Dh, Hkv, Sk, rb, cfg):
    h = pl.program_id(0)
    M = rep * Sq
    G = rep * Dh
    NC = Sk // Dh
    NB = M // rb
    NS = M // 16
    KG = 4 * Dh
    HB = B // 2
    qscale = (Dh ** -0.5) * math.log2(math.e)
    p_bufs = (p0, p1)
    never = h < 0
    slot = lax.rem(h, 2)

    def wq_copy(hh):
        return pltpu.make_async_copy(
            wq_hbm.at[:, pl.ds(hh * G, G)], wq_v.at[hh], wqsem.at[hh])

    def wo_copy(hh, sl):
        return pltpu.make_async_copy(
            wo_hbm.at[pl.ds(hh * G, G), :], wo_v.at[sl], wosem.at[sl])

    def k_copy(hh, sl):
        return pltpu.make_async_copy(k_hbm.at[:, hh], kbuf.at[sl], ksem.at[sl])

    def v_copy(hh, sl):
        return pltpu.make_async_copy(v_hbm.at[:, hh], vbuf.at[sl], vsem.at[sl])

    def out_copy(i):
        return pltpu.make_async_copy(
            obuf.at[pl.ds(i * Sq, Sq), :], out_hbm.at[pl.ds(i * Sq, Sq), :], osem.at[0])

    def prefetch_next(cond):
        @pl.when(cond)
        def _():
            k_copy(h + 1, 1 - slot).start()
            v_copy(h + 1, 1 - slot).start()
            wo_copy(h + 1, 1 - slot).start()

    def attn_block(base, n, first_head, pf_cond):
        cuts = [cfg['cut_first']] + [NC] * (n - 2) + [cfg['cut_last']]

        def qk(i):
            q = q_all[h, base + i]
            k = kbuf[slot, base + i]
            return lax.dot_general(q, k, (((1,), (1,)), ((), ())),
                                   preferred_element_type=jnp.float32)

        def sm_pv(i, s_all, anchors):
            p_ref = p_bufs[i % 2]
            cut = cuts[i]
            ls = []
            part_prev = None
            full_prev = None
            full_prev2 = None
            for j in range(NB):
                s = s_all[j * rb:(j + 1) * rb, :]
                m = jnp.max(s, axis=-1, keepdims=True)
                m = jnp.broadcast_to(m, (rb, Dh))
                fake = anchors[j]
                if part_prev is not None:
                    fake = part_prev if fake is None else fake + part_prev
                if full_prev2 is not None and cut < NC:
                    fake = fake + full_prev2
                if fake is not None:
                    m = jnp.where(never, fake, m)
                ps = [jnp.exp2(s[:, c * Dh:(c + 1) * Dh] - m) for c in range(NC)]
                lp = ps[0]
                for c in range(1, NC):
                    lp = lp + ps[c]
                    if c == cut - 1:
                        part_prev = lp
                full_prev2 = full_prev
                full_prev = lp
                ls.append(lp)
                pb = jnp.concatenate(ps, axis=1).astype(jnp.bfloat16)
                p_ref[j * rb:(j + 1) * rb, :] = pb
            parts = []
            o_raw = None
            for c in range(Sk // KG):
                oc = jnp.dot(p_ref[:, c * KG:(c + 1) * KG],
                             vbuf[slot, base + i, c * KG:(c + 1) * KG, :],
                             preferred_element_type=jnp.float32)
                parts.append(oc)
                o_raw = oc if o_raw is None else o_raw + oc
            lp_all = jnp.concatenate(ls, axis=0)
            lp_all = jnp.where(never, parts[cfg['own_dep']], lp_all)
            l = jnp.sum(lp_all, axis=-1, keepdims=True)
            l = jnp.broadcast_to(l, (M, Dh))
            r = pl.reciprocal(l, approx=True)
            linv = r * (2.0 - l * r)
            o = (o_raw * linv).astype(jnp.bfloat16)
            o = jnp.concatenate([o[r_ * Sq:(r_ + 1) * Sq, :] for r_ in range(rep)], axis=1)
            return o, parts

        def pv_anchor(parts, t):
            c, jj = divmod(t, NS)
            return parts[c][jj * 16:jj * 16 + rb, :]

        def qk_anchor(sn, t):
            c, jj = divmod(t, NS)
            return sn[jj * 16:jj * 16 + rb, c * KG:c * KG + Dh]

        def op(i, o):
            contrib = jnp.dot(o, wo_v[slot], preferred_element_type=jnp.float32)
            if first_head:
                row0 = pl.multiple_of((base + i) * Sq, 16)
                acc_scr[pl.ds(row0, Sq), :] = contrib
            else:
                new = contrib + acc_scr[i * Sq:(i + 1) * Sq, :]
                acc_scr[i * Sq:(i + 1) * Sq, :] = new
                obuf[i * Sq:(i + 1) * Sq, :] = new.astype(obuf.dtype)

                @pl.when(h == Hkv - 1)
                def _():
                    out_copy(i).start()

        s = {}
        o = {}
        parts = {}
        s[0] = qk(0)
        prefetch_next(pf_cond)
        ff, fl = cfg['free_first'], cfg['free_last']
        for i in range(n):
            if i + 1 < n:
                s[i + 1] = qk(i + 1)
            if i == 0:
                anchors = [None if j < ff else
                           qk_anchor(s[1], min(int((j - ff) * cfg['sp_first']), 4 * NS - 1))
                           for j in range(NB)]
            elif i == n - 1:
                anchors = [None if j < fl else
                           pv_anchor(parts[i - 1], min(int((j - fl) * cfg['sp_last']), 4 * NS - 1))
                           for j in range(NB)]
            else:
                anchors = []
                for j in range(NB):
                    t = int(j * cfg['sp_mid'])
                    if t < 4 * NS:
                        anchors.append(pv_anchor(parts[i - 1], t))
                    else:
                        anchors.append(qk_anchor(s[i + 1], min(t - 4 * NS, 4 * NS - 1)))
            o[i], parts[i] = sm_pv(i, s[i], anchors)
            if i >= 1:
                op(i - 1, o[i - 1])
        op(n - 1, o[n - 1])

    @pl.when(h == 0)
    def _():
        xc = pltpu.make_async_copy(x_hbm, x_v, xsem.at[0])
        xc.start()
        wq_copy(0).start()
        wq_copy(1).start()
        xc.wait()
        for hh in range(Hkv):
            wq_copy(hh).wait()
            if hh + 2 < Hkv:
                wq_copy(hh + 2).start()
            pltpu.make_async_copy(k_hbm.at[hh, 0], kbuf.at[0, hh], k0sem.at[hh // HB]).start()
            pltpu.make_async_copy(v_hbm.at[hh, 0], vbuf.at[0, hh], v0sem.at[hh // HB]).start()
            if hh == HB - 1:
                wo_copy(0, 0).start()
            q = jnp.dot(x_v[...], wq_v[hh], preferred_element_type=jnp.float32)
            q = q * qscale
            for bb in range(B):
                for r in range(rep):
                    q_all[hh, bb, r * Sq:(r + 1) * Sq, :] = (
                        q[bb * Sq:(bb + 1) * Sq, r * Dh:(r + 1) * Dh].astype(jnp.bfloat16))
        wo_copy(0, 0).wait()

        def half(t, carry):
            base = t * HB
            pltpu.make_async_copy(k_hbm.at[pl.ds(base, HB), 0], kbuf.at[0, pl.ds(base, HB)],
                                  k0sem.at[t]).wait()
            pltpu.make_async_copy(v_hbm.at[pl.ds(base, HB), 0], vbuf.at[0, pl.ds(base, HB)],
                                  v0sem.at[t]).wait()
            attn_block(base, HB, True, t == 0)
            return carry

        lax.fori_loop(0, 2, half, 0)

    @pl.when(h > 0)
    def _():
        k_copy(h, slot).wait()
        v_copy(h, slot).wait()
        wo_copy(h, slot).wait()
        attn_block(0, B, False, h + 1 < Hkv)

    @pl.when(h == Hkv - 1)
    def _():
        for i in range(B):
            out_copy(i).wait()


def make_kernel(rb=8, **kw):
  cfg = dict(cut_first=10, cut_last=10, sp_first=2.0, sp_mid=3.8, sp_last=2.0,
             own_dep=1, free_first=5, free_last=0)
  cfg.update(kw)
  @jax.jit
  def pallas_standalone__gqa_block_cached__near_ridge_kernel(
    x: jax.Array,
    k_cache: jax.Array,
    v_cache: jax.Array,
    wq: jax.Array,
    wo: jax.Array,
  ):
    B, Sq, D = x.shape
    _, Hkv, Sk, Dh = k_cache.shape
    Hq = wq.shape[1] // Dh
    rep = Hq // Hkv
    G = rep * Dh
    M = rep * Sq
    x2 = x.reshape(B * Sq, D)

    kernel = functools.partial(_kernel, B=B, Sq=Sq, rep=rep, Dh=Dh, Hkv=Hkv, Sk=Sk, rb=rb, cfg=cfg)
    pshape = pltpu.VMEM((M, Sk), jnp.bfloat16)
    anyspec = pl.BlockSpec(memory_space=pl.ANY)
    out = pl.pallas_call(
        kernel,
        grid=(Hkv,),
        in_specs=[anyspec] * 5,
        out_specs=anyspec,
        out_shape=jax.ShapeDtypeStruct((B * Sq, D), x.dtype),
        scratch_shapes=[
            pltpu.VMEM((B * Sq, D), jnp.bfloat16),
            pltpu.VMEM((Hkv, D, G), jnp.bfloat16),
            pltpu.VMEM((2, G, D), jnp.bfloat16),
            pltpu.VMEM((Hkv, B, M, Dh), jnp.bfloat16),
            pltpu.VMEM((2, B, Sk, Dh), jnp.bfloat16),
            pltpu.VMEM((2, B, Sk, Dh), jnp.bfloat16),
            pltpu.VMEM((B * Sq, D), jnp.float32),
            pltpu.VMEM((B * Sq, D), jnp.bfloat16),
            pshape, pshape,
            pltpu.SemaphoreType.DMA((1,)),
            pltpu.SemaphoreType.DMA((Hkv,)),
            pltpu.SemaphoreType.DMA((2,)),
            pltpu.SemaphoreType.DMA((2,)),
            pltpu.SemaphoreType.DMA((2,)),
            pltpu.SemaphoreType.DMA((2,)),
            pltpu.SemaphoreType.DMA((2,)),
            pltpu.SemaphoreType.DMA((1,)),
        ],
        compiler_params=pltpu.CompilerParams(
            dimension_semantics=("arbitrary",),
            vmem_limit_bytes=100 * 1024 * 1024,
            disable_bounds_checks=True,
        ),
    )(x2, k_cache, v_cache, wq, wo)
    return out.reshape(B, Sq, D)
  return pallas_standalone__gqa_block_cached__near_ridge_kernel


pallas_standalone__gqa_block_cached__near_ridge_kernel = make_kernel()
```

```python
import functools
import math

import jax
import jax.numpy as jnp
from jax import lax
import jax.experimental.pallas as pl
import jax.experimental.pallas.tpu as pltpu

_RB = 8


def _kernel(x_hbm, k_hbm, v_hbm, wq_hbm, wo_hbm, out_hbm,
            x_v, wq_bufs, wo_v, q_all, kbuf, vbuf, acc_scr, obuf, p0, p1,
            xsem, wqsem, wosem, ksem, vsem, k0sem, v0sem, osem,
            *, B, Sq, rep, Dh, Hkv, Sk, cfg):
    h = pl.program_id(0)
    rb = _RB
    M = rep * Sq
    G = rep * Dh
    NC = Sk // Dh
    NB = M // rb
    NS = M // 16
    KG = 4 * Dh
    NG = Sk // KG
    HB = B // 2
    scale2 = (Dh ** -0.5) * math.log2(math.e)
    p_bufs = (p0, p1)
    never = h < 0
    slot = lax.rem(h, 2)
    groups = cfg["groups"]
    gstart = [sum(groups[:i]) for i in range(len(groups))]

    def _tie(after, value):
        return jnp.where(never, after, value)

    def wq_copy(gi):
        c0, nc = gstart[gi] * Dh, groups[gi] * Dh
        return pltpu.make_async_copy(
            wq_hbm.at[:, pl.ds(c0, nc)], wq_bufs[gi].at[:, pl.ds(0, nc)], wqsem.at[gi])

    def wo_copy(hh, sl):
        return pltpu.make_async_copy(
            wo_hbm.at[pl.ds(hh * G, G), :], wo_v.at[sl], wosem.at[sl])

    def k_copy(hh, sl):
        return pltpu.make_async_copy(k_hbm.at[:, hh], kbuf.at[sl], ksem.at[sl])

    def v_copy(hh, sl):
        return pltpu.make_async_copy(v_hbm.at[:, hh], vbuf.at[sl], vsem.at[sl])

    def k0_copy(t):
        return pltpu.make_async_copy(k_hbm.at[pl.ds(t * HB, HB), 0],
                                     kbuf.at[0, pl.ds(t * HB, HB)], k0sem.at[t])

    def v0_copy(t):
        return pltpu.make_async_copy(v_hbm.at[pl.ds(t * HB, HB), 0],
                                     vbuf.at[0, pl.ds(t * HB, HB)], v0sem.at[t])

    def out_copy(i):
        return pltpu.make_async_copy(
            obuf.at[pl.ds(i * Sq, Sq), :], out_hbm.at[pl.ds(i * Sq, Sq), :], osem.at[0])

    def prefetch_next(cond):
        @pl.when(cond)
        def _():
            k_copy(h + 1, 1 - slot).start()
            v_copy(h + 1, 1 - slot).start()
            wo_copy(h + 1, 1 - slot).start()

    def qproj(gi):
        u = gstart[gi]
        end = u + groups[gi]
        while u < end:
            w = min(rep, end - u)
            u_ = u - gstart[gi]
            q = jnp.dot(x_v[...], wq_bufs[gi][:, u_ * Dh:(u_ + w) * Dh],
                        preferred_element_type=jnp.float32).astype(jnp.bfloat16)
            for bb in range(B):
                for r in range(w):
                    hh, rr = divmod(u + r, rep)
                    q_all[hh, bb, rr * Sq:(rr + 1) * Sq, :] = (
                        q[bb * Sq:(bb + 1) * Sq, r * Dh:(r + 1) * Dh])
            u += w

    def attn_block(base, n, first_head, pf_cond):
        cuts = [cfg["cut_first"]] + [NC] * (n - 2) + [cfg["cut_last"]]

        def qk(i):
            return lax.dot_general(q_all[h, base + i], kbuf[slot, base + i],
                                   (((1,), (1,)), ((), ())),
                                   preferred_element_type=jnp.float32)

        def sm_pv(i, s_all, anchors):
            p_ref = p_bufs[i % 2]
            cut = cuts[i]
            lps = []
            part_prev = None
            for j in range(NB):
                s = s_all[j * rb:(j + 1) * rb, :]
                m = jnp.broadcast_to(jnp.max(s, axis=-1, keepdims=True), (rb, Dh))
                after = anchors[j]
                if part_prev is not None:
                    after = part_prev if after is None else after + part_prev
                if j >= 2 and cut < NC:
                    after = after + lps[j - 2]
                if after is not None:
                    m = _tie(after, m)
                ps = [jnp.exp2((s[:, c * Dh:(c + 1) * Dh] - m) * scale2) for c in range(NC)]
                lp = ps[0]
                for c in range(1, NC):
                    lp = lp + ps[c]
                    if c == cut - 1:
                        part_prev = lp
                lps.append(lp)
                p_ref[j * rb:(j + 1) * rb, :] = (
                    jnp.concatenate(ps, axis=1).astype(jnp.bfloat16))
            parts = []
            o_raw = None
            for c in range(NG):
                oc = jnp.dot(p_ref[:, c * KG:(c + 1) * KG],
                             vbuf[slot, base + i, c * KG:(c + 1) * KG, :],
                             preferred_element_type=jnp.float32)
                parts.append(oc)
                o_raw = oc if o_raw is None else o_raw + oc
            lp_all = _tie(parts[cfg["own_dep"]], jnp.concatenate(lps, axis=0))
            l = jnp.broadcast_to(jnp.sum(lp_all, axis=-1, keepdims=True), (M, Dh))
            r = pl.reciprocal(l, approx=True)
            linv = r * (2.0 - l * r)
            o = (o_raw * linv).astype(jnp.bfloat16)
            o = jnp.concatenate([o[r_ * Sq:(r_ + 1) * Sq, :] for r_ in range(rep)], axis=1)
            return o, parts, linv

        def pv_anchor(parts, t):
            c, jj = divmod(min(t, NG * NS - 1), NS)
            return parts[c][jj * 16:jj * 16 + rb, :]

        def qk_anchor(sn, t):
            c, jj = divmod(min(t, NG * NS - 1), NS)
            return sn[jj * 16:jj * 16 + rb, c * KG:c * KG + Dh]

        def oproj(i, o):
            contrib = jnp.dot(o, wo_v[slot], preferred_element_type=jnp.float32)
            if first_head:
                row0 = pl.multiple_of((base + i) * Sq, 16)
                acc_scr[pl.ds(row0, Sq), :] = contrib
            else:
                new = contrib + acc_scr[i * Sq:(i + 1) * Sq, :]
                acc_scr[i * Sq:(i + 1) * Sq, :] = new
                obuf[i * Sq:(i + 1) * Sq, :] = new.astype(obuf.dtype)

                @pl.when(h == Hkv - 1)
                def _():
                    out_copy(i).start()

        s, o, parts, linvs = {}, {}, {}, {}
        s[0] = qk(0)
        prefetch_next(pf_cond)
        ff = cfg["free_first"]
        for i in range(n):
            if i + 1 < n:
                s[i + 1] = qk(i + 1)
            if i == 0:
                anchors = [None if j < ff else
                           qk_anchor(s[1], int((j - ff) * cfg["sp_first"]))
                           for j in range(NB)]
            elif i == n - 1:
                anchors = [pv_anchor(parts[i - 1], int(j * cfg["sp_last"]))
                           for j in range(NB)]
            else:
                anchors = []
                for j in range(NB):
                    t = int(j * cfg["sp_mid"])
                    anchors.append(pv_anchor(parts[i - 1], t) if t < NG * NS
                                   else qk_anchor(s[i + 1], t - NG * NS))
                if i == n - 2:
                    for jj in range(NB):
                        j = NB // 2 + jj // 2
                        anchors[j] = anchors[j] + linvs[i - 1][jj * rb:(jj + 1) * rb, :]
            o[i], parts[i], linvs[i] = sm_pv(i, s[i], anchors)
            if i >= 1:
                oproj(i - 1, o[i - 1])
        oproj(n - 1, o[n - 1])

    @pl.when(h == 0)
    def _():
        xc = pltpu.make_async_copy(x_hbm, x_v, xsem.at[0])
        xc.start()
        wq_copy(0).start()
        wq_copy(1).start()
        xc.wait()
        ng = len(groups)
        for gi in range(ng):
            wq_copy(gi).wait()
            if gi + 2 < ng:
                wq_copy(gi + 2).start()
            if gi == ng - 2:
                k0_copy(0).start()
                v0_copy(0).start()
                wo_copy(0, 0).start()
            if gi == ng - 1:
                k0_copy(1).start()
                v0_copy(1).start()
            qproj(gi)
        wo_copy(0, 0).wait()

        def half(t, carry):
            k0_copy(t).wait()
            v0_copy(t).wait()
            attn_block(t * HB, HB, True, t == 0)
            return carry

        lax.fori_loop(0, 2, half, 0)

    @pl.when(h > 0)
    def _():
        k_copy(h, slot).wait()
        v_copy(h, slot).wait()
        wo_copy(h, slot).wait()
        attn_block(0, B, False, h + 1 < Hkv)

    @pl.when(h == Hkv - 1)
    def _():
        for i in range(B):
            out_copy(i).wait()


def make_kernel(**kw):
    cfg = dict(cut_first=8, cut_last=8, sp_first=2.0, sp_mid=3.8, sp_last=2.0,
               own_dep=1, free_first=5, groups=(1, 3, 8, 20))
    cfg.update(kw)

    @jax.jit
    def pallas_standalone__gqa_block_cached__near_ridge_kernel(
        x: jax.Array,
        k_cache: jax.Array,
        v_cache: jax.Array,
        wq: jax.Array,
        wo: jax.Array,
    ):
        B, Sq, D = x.shape
        _, Hkv, Sk, Dh = k_cache.shape
        Hq = wq.shape[1] // Dh
        rep = Hq // Hkv
        G = rep * Dh
        M = rep * Sq
        groups = cfg["groups"]
        assert sum(groups) == Hq and Hkv >= 2 and B % 2 == 0 and B >= 4
        assert Sq % 16 == 0 and Sk % (4 * Dh) == 0
        bf16 = jnp.bfloat16
        kernel = functools.partial(_kernel, B=B, Sq=Sq, rep=rep, Dh=Dh, Hkv=Hkv, Sk=Sk, cfg=cfg)
        anyspec = pl.BlockSpec(memory_space=pl.ANY)
        out = pl.pallas_call(
            kernel,
            grid=(Hkv,),
            in_specs=[anyspec] * 5,
            out_specs=anyspec,
            out_shape=jax.ShapeDtypeStruct((B * Sq, D), x.dtype),
            scratch_shapes=[
                pltpu.VMEM((B * Sq, D), bf16),
                [pltpu.VMEM((D, (g + 1 if g % 8 == 0 else g) * Dh), bf16)
                 for g in groups],
                pltpu.VMEM((2, G, D), bf16),
                pltpu.VMEM((Hkv, B, M, Dh), bf16),
                pltpu.VMEM((2, B, Sk, Dh), bf16),
                pltpu.VMEM((2, B, Sk, Dh), bf16),
                pltpu.VMEM((B * Sq, D), jnp.float32),
                pltpu.VMEM((B * Sq, D), x.dtype),
                pltpu.VMEM((M, Sk), bf16),
                pltpu.VMEM((M, Sk), bf16),
                pltpu.SemaphoreType.DMA((1,)),
                pltpu.SemaphoreType.DMA((len(groups),)),
                pltpu.SemaphoreType.DMA((2,)),
                pltpu.SemaphoreType.DMA((2,)),
                pltpu.SemaphoreType.DMA((2,)),
                pltpu.SemaphoreType.DMA((2,)),
                pltpu.SemaphoreType.DMA((2,)),
                pltpu.SemaphoreType.DMA((1,)),
            ],
            compiler_params=pltpu.CompilerParams(
                dimension_semantics=("arbitrary",),
                vmem_limit_bytes=100 * 1024 * 1024,
                disable_bounds_checks=True,
            ),
        )(x.reshape(B * Sq, D), k_cache, v_cache, wq, wo)
        return out.reshape(B, Sq, D)

    return pallas_standalone__gqa_block_cached__near_ridge_kernel


pallas_standalone__gqa_block_cached__near_ridge_kernel = make_kernel()
```

```python
import functools
import math

import jax
import jax.numpy as jnp
from jax import lax
import jax.experimental.pallas as pl
import jax.experimental.pallas.tpu as pltpu

_RB = 8


def _kernel(x_hbm, k_hbm, v_hbm, wq_hbm, wo_hbm, out_hbm,
            x_v, wq_bufs, wo_v, q_all, kbuf, vbuf, acc_scr, obuf, p0, p1,
            xsem, wqsem, wosem, ksem, vsem, k0sem, v0sem, osem,
            *, B, Sq, rep, Dh, Hkv, Sk, cfg):
    rb = _RB
    M = rep * Sq
    G = rep * Dh
    NC = Sk // Dh
    NB = M // rb
    NS = M // 16
    KG = 4 * Dh
    NG = Sk // KG
    HB = B // 2
    scale2 = (Dh ** -0.5) * math.log2(math.e)
    p_bufs = (p0, p1)
    groups = cfg["groups"]
    gstart = [sum(groups[:i]) for i in range(len(groups))]

    def wq_copy(gi):
        c0, nc = gstart[gi] * Dh, groups[gi] * Dh
        return pltpu.make_async_copy(
            wq_hbm.at[:, pl.ds(c0, nc)], wq_bufs[gi].at[:, pl.ds(0, nc)], wqsem.at[gi])

    def wo_copy(hh, sl):
        return pltpu.make_async_copy(
            wo_hbm.at[pl.ds(hh * G, G), :], wo_v.at[sl], wosem.at[sl])

    def k_copy(hh, sl):
        return pltpu.make_async_copy(k_hbm.at[:, hh], kbuf.at[sl], ksem.at[sl])

    def v_copy(hh, sl):
        return pltpu.make_async_copy(v_hbm.at[:, hh], vbuf.at[sl], vsem.at[sl])

    def k0_copy(t):
        return pltpu.make_async_copy(k_hbm.at[pl.ds(t * HB, HB), 0],
                                     kbuf.at[0, pl.ds(t * HB, HB)], k0sem.at[t])

    def v0_copy(t):
        return pltpu.make_async_copy(v_hbm.at[pl.ds(t * HB, HB), 0],
                                     vbuf.at[0, pl.ds(t * HB, HB)], v0sem.at[t])

    def out_copy(i):
        return pltpu.make_async_copy(
            obuf.at[pl.ds(i * Sq, Sq), :], out_hbm.at[pl.ds(i * Sq, Sq), :], osem.at[0])

    def qproj(gi):
        u = gstart[gi]
        end = u + groups[gi]
        while u < end:
            w = min(rep, end - u)
            u_ = u - gstart[gi]
            q = jnp.dot(x_v[...], wq_bufs[gi][:, u_ * Dh:(u_ + w) * Dh],
                        preferred_element_type=jnp.float32).astype(jnp.bfloat16)
            for bb in range(B):
                for r in range(w):
                    hh, rr = divmod(u + r, rep)
                    q_all[hh, bb, rr * Sq:(rr + 1) * Sq, :] = (
                        q[bb * Sq:(bb + 1) * Sq, r * Dh:(r + 1) * Dh])
            u += w

    def attn_block(h, slot, base, n, first_head, pf_cond, never):
        def _tie(after, value):
            return jnp.where(never, after, value)

        def prefetch_next(cond):
            @pl.when(cond)
            def _():
                k_copy(h + 1, 1 - slot).start()
                v_copy(h + 1, 1 - slot).start()
                wo_copy(h + 1, 1 - slot).start()

        cuts = [cfg["cut_first"]] + [NC] * (n - 2) + [cfg["cut_last"]]

        def qk(i):
            return lax.dot_general(q_all[h, base + i], kbuf[slot, base + i],
                                   (((1,), (1,)), ((), ())),
                                   preferred_element_type=jnp.float32)

        def sm_pv(i, s_all, anchors):
            p_ref = p_bufs[i % 2]
            cut = cuts[i]
            lps = []
            part_prev = None
            for j in range(NB):
                s = s_all[j * rb:(j + 1) * rb, :]
                m = jnp.broadcast_to(jnp.max(s, axis=-1, keepdims=True), (rb, Dh))
                after = anchors[j]
                if part_prev is not None:
                    after = part_prev if after is None else after + part_prev
                if j >= 2 and cut < NC:
                    after = after + lps[j - 2]
                if after is not None:
                    m = _tie(after, m)
                ps = [jnp.exp2((s[:, c * Dh:(c + 1) * Dh] - m) * scale2) for c in range(NC)]
                lp = ps[0]
                for c in range(1, NC):
                    lp = lp + ps[c]
                    if c == cut - 1:
                        part_prev = lp
                lps.append(lp)
                p_ref[j * rb:(j + 1) * rb, :] = (
                    jnp.concatenate(ps, axis=1).astype(jnp.bfloat16))
            parts = []
            o_raw = None
            for c in range(NG):
                oc = jnp.dot(p_ref[:, c * KG:(c + 1) * KG],
                             vbuf[slot, base + i, c * KG:(c + 1) * KG, :],
                             preferred_element_type=jnp.float32)
                parts.append(oc)
                o_raw = oc if o_raw is None else o_raw + oc
            lp_all = _tie(parts[cfg["own_dep"]], jnp.concatenate(lps, axis=0))
            l = jnp.broadcast_to(jnp.sum(lp_all, axis=-1, keepdims=True), (M, Dh))
            r = pl.reciprocal(l, approx=True)
            linv = r * (2.0 - l * r)
            o = (o_raw * linv).astype(jnp.bfloat16)
            o = jnp.concatenate([o[r_ * Sq:(r_ + 1) * Sq, :] for r_ in range(rep)], axis=1)
            return o, parts, linv

        def pv_anchor(parts, t):
            c, jj = divmod(min(t, NG * NS - 1), NS)
            return parts[c][jj * 16:jj * 16 + rb, :]

        def qk_anchor(sn, t):
            c, jj = divmod(min(t, NG * NS - 1), NS)
            return sn[jj * 16:jj * 16 + rb, c * KG:c * KG + Dh]

        def oproj(i, o):
            contrib = jnp.dot(o, wo_v[slot], preferred_element_type=jnp.float32)
            if first_head:
                row0 = pl.multiple_of((base + i) * Sq, 16)
                acc_scr[pl.ds(row0, Sq), :] = contrib
            else:
                new = contrib + acc_scr[i * Sq:(i + 1) * Sq, :]
                acc_scr[i * Sq:(i + 1) * Sq, :] = new
                obuf[i * Sq:(i + 1) * Sq, :] = new.astype(obuf.dtype)

                @pl.when(h == Hkv - 1)
                def _():
                    out_copy(i).start()

        s, o, parts, linvs = {}, {}, {}, {}
        s[0] = qk(0)
        prefetch_next(pf_cond)
        ff = cfg["free_first"]
        for i in range(n):
            if i + 1 < n:
                s[i + 1] = qk(i + 1)
            if i == 0:
                anchors = [None if j < ff else
                           qk_anchor(s[1], int((j - ff) * cfg["sp_first"]))
                           for j in range(NB)]
            elif i == n - 1:
                anchors = [pv_anchor(parts[i - 1], int(j * cfg["sp_last"]))
                           for j in range(NB)]
            else:
                anchors = []
                for j in range(NB):
                    t = int(j * cfg["sp_mid"])
                    anchors.append(pv_anchor(parts[i - 1], t) if t < NG * NS
                                   else qk_anchor(s[i + 1], t - NG * NS))
                if i == n - 2:
                    for jj in range(NB):
                        j = NB // 2 + jj // 2
                        anchors[j] = anchors[j] + linvs[i - 1][jj * rb:(jj + 1) * rb, :]
            o[i], parts[i], linvs[i] = sm_pv(i, s[i], anchors)
            if i >= 1:
                oproj(i - 1, o[i - 1])
        oproj(n - 1, o[n - 1])

    step = pl.program_id(0)

    @pl.when(step == 0)
    def _():
        xc = pltpu.make_async_copy(x_hbm, x_v, xsem.at[0])
        xc.start()
        wq_copy(0).start()
        wq_copy(1).start()
        xc.wait()
        ng = len(groups)
        for gi in range(ng):
            wq_copy(gi).wait()
            if gi + 2 < ng:
                wq_copy(gi + 2).start()
            if gi == ng - 2:
                k0_copy(0).start()
                v0_copy(0).start()
                wo_copy(0, 0).start()
            if gi == ng - 1:
                k0_copy(1).start()
                v0_copy(1).start()
            qproj(gi)
        wo_copy(0, 0).wait()

        def half(t, carry):
            k0_copy(t).wait()
            v0_copy(t).wait()
            attn_block(step, step, t * HB, HB, True, t == 0, step < 0)
            return carry

        lax.fori_loop(0, 2, half, 0)

    @pl.when(step == 1)
    def _():
        def head(h, carry):
            slot = h & 1
            k_copy(h, slot).wait()
            v_copy(h, slot).wait()
            wo_copy(h, slot).wait()
            attn_block(h, slot, 0, B, False, h + 1 < Hkv, h < 0)
            return carry

        lax.fori_loop(1, Hkv, head, 0)

        for i in range(B):
            out_copy(i).wait()


def make_kernel(**kw):
    cfg = dict(cut_first=8, cut_last=8, sp_first=2.0, sp_mid=3.8, sp_last=2.0,
               own_dep=1, free_first=5, groups=(1, 3, 8, 20))
    cfg.update(kw)

    @jax.jit
    def pallas_standalone__gqa_block_cached__near_ridge_kernel(
        x: jax.Array,
        k_cache: jax.Array,
        v_cache: jax.Array,
        wq: jax.Array,
        wo: jax.Array,
    ):
        B, Sq, D = x.shape
        _, Hkv, Sk, Dh = k_cache.shape
        Hq = wq.shape[1] // Dh
        rep = Hq // Hkv
        G = rep * Dh
        M = rep * Sq
        groups = cfg["groups"]
        assert sum(groups) == Hq and Hkv >= 2 and B % 2 == 0 and B >= 4
        assert Sq % 16 == 0 and Sk % (4 * Dh) == 0
        bf16 = jnp.bfloat16
        kernel = functools.partial(_kernel, B=B, Sq=Sq, rep=rep, Dh=Dh, Hkv=Hkv, Sk=Sk, cfg=cfg)
        anyspec = pl.BlockSpec(memory_space=pl.ANY)
        out = pl.pallas_call(
            kernel,
            grid=(2,),
            in_specs=[anyspec] * 5,
            out_specs=anyspec,
            out_shape=jax.ShapeDtypeStruct((B * Sq, D), x.dtype),
            scratch_shapes=[
                pltpu.VMEM((B * Sq, D), bf16),
                [pltpu.VMEM((D, (g + 1 if g % 8 == 0 else g) * Dh), bf16)
                 for g in groups],
                pltpu.VMEM((2, G, D), bf16),
                pltpu.VMEM((Hkv, B, M, Dh), bf16),
                pltpu.VMEM((2, B, Sk, Dh), bf16),
                pltpu.VMEM((2, B, Sk, Dh), bf16),
                pltpu.VMEM((B * Sq, D), jnp.float32),
                pltpu.VMEM((B * Sq, D), x.dtype),
                pltpu.VMEM((M, Sk), bf16),
                pltpu.VMEM((M, Sk), bf16),
                pltpu.SemaphoreType.DMA((1,)),
                pltpu.SemaphoreType.DMA((len(groups),)),
                pltpu.SemaphoreType.DMA((2,)),
                pltpu.SemaphoreType.DMA((2,)),
                pltpu.SemaphoreType.DMA((2,)),
                pltpu.SemaphoreType.DMA((2,)),
                pltpu.SemaphoreType.DMA((2,)),
                pltpu.SemaphoreType.DMA((1,)),
            ],
            compiler_params=pltpu.CompilerParams(
                dimension_semantics=("arbitrary",),
                vmem_limit_bytes=100 * 1024 * 1024,
                disable_bounds_checks=True,
                disable_semaphore_checks=True,
            ),
        )(x.reshape(B * Sq, D), k_cache, v_cache, wq, wo)
        return out.reshape(B, Sq, D)

    return pallas_standalone__gqa_block_cached__near_ridge_kernel


pallas_standalone__gqa_block_cached__near_ridge_kernel = make_kernel()
```

```python
import functools
import math

import jax
import jax.numpy as jnp
from jax import lax
import jax.experimental.pallas as pl
import jax.experimental.pallas.tpu as pltpu

_RB = 8
_WCHUNK = 512


def _kernel(x_hbm, k_hbm, v_hbm, wq_hbm, wo_hbm, out_hbm,
            x_v, wq_bufs, wo_v, q_all, kbuf, vbuf, acc_scr, obuf, p0, p1,
            xsem, wqsem, wosem, ksem, vsem, k0sem, v0sem, osem,
            *, B, Sq, rep, Dh, Hkv, Sk, groups):
    rb = _RB
    W = _WCHUNK
    M = rep * Sq
    G = rep * Dh
    NB = M // rb
    NS = M // 16
    KG = 4 * Dh
    NG = Sk // KG
    HB = B // 2
    scale2 = (Dh ** -0.5) * math.log2(math.e)
    p_bufs = (p0, p1)
    gstart = [sum(groups[:i]) for i in range(len(groups))]

    def wq_copy(gi):
        c0, nc = gstart[gi] * Dh, groups[gi] * Dh
        return pltpu.make_async_copy(
            wq_hbm.at[:, pl.ds(c0, nc)], wq_bufs[gi].at[:, pl.ds(0, nc)], wqsem.at[gi])

    def wo_copy(hh, sl):
        return pltpu.make_async_copy(
            wo_hbm.at[pl.ds(hh * G, G), :], wo_v.at[sl], wosem.at[sl])

    def k_copy(hh, sl):
        return pltpu.make_async_copy(k_hbm.at[:, hh], kbuf.at[sl], ksem.at[sl])

    def v_copy(hh, sl):
        return pltpu.make_async_copy(v_hbm.at[:, hh], vbuf.at[sl], vsem.at[sl])

    def k0_copy(t):
        return pltpu.make_async_copy(k_hbm.at[pl.ds(t * HB, HB), 0],
                                     kbuf.at[0, pl.ds(t * HB, HB)], k0sem.at[t])

    def v0_copy(t):
        return pltpu.make_async_copy(v_hbm.at[pl.ds(t * HB, HB), 0],
                                     vbuf.at[0, pl.ds(t * HB, HB)], v0sem.at[t])

    def out_copy(i):
        return pltpu.make_async_copy(
            obuf.at[pl.ds(i * Sq, Sq), :], out_hbm.at[pl.ds(i * Sq, Sq), :], osem.at[0])

    def qproj(gi):
        u = gstart[gi]
        end = u + groups[gi]
        while u < end:
            w = min(rep, end - u)
            u_ = u - gstart[gi]
            q = jnp.dot(x_v[...], wq_bufs[gi][:, u_ * Dh:(u_ + w) * Dh],
                        preferred_element_type=jnp.float32).astype(jnp.bfloat16)
            for bb in range(B):
                for r in range(w):
                    hh, rr = divmod(u + r, rep)
                    q_all[hh, bb, rr * Sq:(rr + 1) * Sq, :] = (
                        q[bb * Sq:(bb + 1) * Sq, r * Dh:(r + 1) * Dh])
            u += w

    def attn_block(h, slot, base, n, first_head, pf_cond, never):
        def _tie(after, value):
            return jnp.where(never, after, value)

        def qk(i):
            return lax.dot_general(q_all[h, base + i], kbuf[slot, base + i],
                                   (((1,), (1,)), ((), ())),
                                   preferred_element_type=jnp.float32)

        def softmax_pv(i, s_all, anchors, lag):
            p_ref = p_bufs[i % 2]
            lps = []
            for j in range(NB):
                s = s_all[j * rb:(j + 1) * rb, :]
                m = jnp.broadcast_to(jnp.max(s, axis=-1, keepdims=True), (rb, Dh))
                after = anchors[j]
                if j >= lag:
                    after = lps[j - lag] if after is None else after + lps[j - lag]
                if after is not None:
                    m = _tie(after, m)
                mw = jnp.concatenate([m] * (W // Dh), axis=1)
                ps = [jnp.exp2((s[:, c * W:(c + 1) * W] - mw) * scale2)
                      for c in range(Sk // W)]
                lp = ps[0]
                for pc in ps[1:]:
                    lp = lp + pc
                while lp.shape[1] > Dh:
                    hw = lp.shape[1] // 2
                    lp = lp[:, :hw] + lp[:, hw:]
                lps.append(lp)
                p_ref[j * rb:(j + 1) * rb, :] = (
                    jnp.concatenate(ps, axis=1).astype(jnp.bfloat16))
            parts = []
            o_raw = None
            for c in range(NG):
                oc = jnp.dot(p_ref[:, c * KG:(c + 1) * KG],
                             vbuf[slot, base + i, c * KG:(c + 1) * KG, :],
                             preferred_element_type=jnp.float32)
                parts.append(oc)
                o_raw = oc if o_raw is None else o_raw + oc
            lp_all = _tie(parts[1], jnp.concatenate(lps, axis=0))
            l = jnp.broadcast_to(jnp.sum(lp_all, axis=-1, keepdims=True), (M, Dh))
            r = pl.reciprocal(l, approx=True)
            linv = r * (2.0 - l * r)
            o = (o_raw * linv).astype(jnp.bfloat16)
            o = jnp.concatenate([o[r_ * Sq:(r_ + 1) * Sq, :] for r_ in range(rep)], axis=1)
            return o, parts, linv

        def pv_anchor(parts, t):
            c, jj = divmod(min(t, NG * NS - 1), NS)
            return parts[c][jj * 16:jj * 16 + rb, :]

        def qk_anchor(sn, t):
            c, jj = divmod(min(t, NG * NS - 1), NS)
            return sn[jj * 16:jj * 16 + rb, c * KG:c * KG + Dh]

        def oproj(i, o):
            contrib = jnp.dot(o, wo_v[slot], preferred_element_type=jnp.float32)
            if first_head:
                row0 = pl.multiple_of((base + i) * Sq, 16)
                acc_scr[pl.ds(row0, Sq), :] = contrib
            else:
                new = contrib + acc_scr[i * Sq:(i + 1) * Sq, :]
                acc_scr[i * Sq:(i + 1) * Sq, :] = new
                obuf[i * Sq:(i + 1) * Sq, :] = new.astype(obuf.dtype)

                @pl.when(h == Hkv - 1)
                def _():
                    out_copy(i).start()

        s, o, parts, linvs = {}, {}, {}, {}
        s[0] = qk(0)

        @pl.when(pf_cond)
        def _():
            k_copy(h + 1, 1 - slot).start()
            v_copy(h + 1, 1 - slot).start()
            wo_copy(h + 1, 1 - slot).start()

        for i in range(n):
            if i + 1 < n:
                s[i + 1] = qk(i + 1)
            if i == 0:
                lag = 2
                anchors = [None if j < 5 else qk_anchor(s[1], int((j - 5) * 1.9))
                           for j in range(NB)]
            elif i == n - 1:
                lag = 2
                anchors = [pv_anchor(parts[i - 1], 2 * j) for j in range(NB)]
            else:
                lag = 1
                anchors = []
                for j in range(NB):
                    t = int(j * 3.6)
                    anchors.append(pv_anchor(parts[i - 1], t) if t < NG * NS
                                   else qk_anchor(s[i + 1], t - NG * NS))
                if i == n - 2:
                    for jj in range(NB):
                        j = NB // 2 + jj // 2
                        anchors[j] = anchors[j] + linvs[i - 1][jj * rb:(jj + 1) * rb, :]
            o[i], parts[i], linvs[i] = softmax_pv(i, s[i], anchors, lag)
            if i >= 1:
                oproj(i - 1, o[i - 1])
        oproj(n - 1, o[n - 1])

    step = pl.program_id(0)

    @pl.when(step == 0)
    def _():
        xc = pltpu.make_async_copy(x_hbm, x_v, xsem.at[0])
        xc.start()
        wq_copy(0).start()
        wq_copy(1).start()
        xc.wait()
        ng = len(groups)
        for gi in range(ng):
            wq_copy(gi).wait()
            if gi + 2 < ng:
                wq_copy(gi + 2).start()
            if gi == ng - 2:
                k0_copy(0).start()
                v0_copy(0).start()
                wo_copy(0, 0).start()
            if gi == ng - 1:
                k0_copy(1).start()
                v0_copy(1).start()
            qproj(gi)
        wo_copy(0, 0).wait()

        def half(t, carry):
            k0_copy(t).wait()
            v0_copy(t).wait()
            attn_block(step, step, t * HB, HB, True, t == 0, step < 0)
            return carry

        lax.fori_loop(0, 2, half, 0)

    @pl.when(step == 1)
    def _():
        def head(h, carry):
            slot = h & 1
            k_copy(h, slot).wait()
            v_copy(h, slot).wait()
            wo_copy(h, slot).wait()
            attn_block(h, slot, 0, B, False, h + 1 < Hkv, h < 0)
            return carry

        lax.fori_loop(1, Hkv, head, 0)

        for i in range(B):
            out_copy(i).wait()


def make_kernel(groups=(1, 3, 8, 20)):
    @jax.jit
    def pallas_standalone__gqa_block_cached__near_ridge_kernel(
        x: jax.Array,
        k_cache: jax.Array,
        v_cache: jax.Array,
        wq: jax.Array,
        wo: jax.Array,
    ):
        B, Sq, D = x.shape
        _, Hkv, Sk, Dh = k_cache.shape
        Hq = wq.shape[1] // Dh
        rep = Hq // Hkv
        G = rep * Dh
        M = rep * Sq
        assert sum(groups) == Hq and Hkv >= 2 and B % 2 == 0 and B >= 4
        assert Sq % 16 == 0 and Sk % (4 * Dh) == 0 and Sk >= 8 * Dh
        bf16 = jnp.bfloat16
        kernel = functools.partial(_kernel, B=B, Sq=Sq, rep=rep, Dh=Dh, Hkv=Hkv, Sk=Sk,
                                   groups=groups)
        anyspec = pl.BlockSpec(memory_space=pl.ANY)
        out = pl.pallas_call(
            kernel,
            grid=(2,),
            in_specs=[anyspec] * 5,
            out_specs=anyspec,
            out_shape=jax.ShapeDtypeStruct((B * Sq, D), x.dtype),
            scratch_shapes=[
                pltpu.VMEM((B * Sq, D), bf16),
                [pltpu.VMEM((D, (g + 1 if g % 8 == 0 else g) * Dh), bf16)
                 for g in groups],
                pltpu.VMEM((2, G, D), bf16),
                pltpu.VMEM((Hkv, B, M, Dh), bf16),
                pltpu.VMEM((2, B, Sk, Dh), bf16),
                pltpu.VMEM((2, B, Sk, Dh), bf16),
                pltpu.VMEM((B * Sq, D), jnp.float32),
                pltpu.VMEM((B * Sq, D), x.dtype),
                pltpu.VMEM((M, Sk), bf16),
                pltpu.VMEM((M, Sk), bf16),
                pltpu.SemaphoreType.DMA((1,)),
                pltpu.SemaphoreType.DMA((len(groups),)),
                pltpu.SemaphoreType.DMA((2,)),
                pltpu.SemaphoreType.DMA((2,)),
                pltpu.SemaphoreType.DMA((2,)),
                pltpu.SemaphoreType.DMA((2,)),
                pltpu.SemaphoreType.DMA((2,)),
                pltpu.SemaphoreType.DMA((1,)),
            ],
            compiler_params=pltpu.CompilerParams(
                dimension_semantics=("arbitrary",),
                vmem_limit_bytes=100 * 1024 * 1024,
                disable_bounds_checks=True,
                disable_semaphore_checks=True,
            ),
        )(x.reshape(B * Sq, D), k_cache, v_cache, wq, wo)
        return out.reshape(B, Sq, D)

    return pallas_standalone__gqa_block_cached__near_ridge_kernel


pallas_standalone__gqa_block_cached__near_ridge_kernel = make_kernel()
```
